```python
import jax
import jax.numpy as jnp

def _softmax(x, axis=-1):
    return jax.nn.softmax(x, axis=axis)
def _gelu(x):
    return jax.nn.gelu(x, approximate=True)
def _silu(x):
    return jax.nn.silu(x)
def _sigmoid(x):
    return jax.nn.sigmoid(x)
def _layernorm(x, axis=-1, eps=1e-5):
    m = jnp.mean(x, axis=axis, keepdims=True)
    v = jnp.var(x, axis=axis, keepdims=True)
    return (x - m) / jnp.sqrt(v + eps)
def _scatter_add(tgt, idx, src, axis=0):
    return tgt.at[idx].add(src)
def _segment_sum(src, seg, n):
    return jax.ops.segment_sum(src, seg, n)
class _Rng:
    def __init__(self, key):
        self._k = key
    def _next(self):
        self._k, sub = jax.random.split(self._k)
        return sub
    def normal(self, shape):
        return jax.random.normal(self._next(), shape, dtype=jnp.bfloat16)
    def randint(self, lo, hi, shape):
        return jax.random.randint(self._next(), shape, lo, hi, dtype=jnp.int32)
    def uniform(self, shape, lo=0.0, hi=1.0):
        return jax.random.uniform(self._next(), shape, jnp.bfloat16, lo, hi)
    def permutation(self, n):
        return jax.random.permutation(self._next(), n)


kernel_name = 'standalone__cross_network_dcn__recsys'

def setup_inputs():
    _rng = _Rng(jax.random.key(int.from_bytes(__import__("os").urandom(4), "little")))
    _w = (lambda a: (lambda t: t.astype(jnp.bfloat16) if jnp.issubdtype(t.dtype, jnp.floating) else t)(jnp.asarray(a)))
    B, F, D, L = 16384, 100, 16, 6
    Din = min(F * D, 1024)
    return {
        "x0": _w((lambda *s: _rng.normal(s) * 0.05)(B, Din)),
        "ws": _w((lambda *s: _rng.normal(s) * 0.05)(L, Din, Din) * (Din ** -0.5)),
        "bs": _w((lambda *s: _rng.normal(s) * 0.05)(L, Din) * 0.01),
    }

def reference(x0, ws, bs):
    x = x0
    L = ws.shape[0]
    for l in range(L):
        proj = jnp.einsum('bd,de->be', x, ws[l]) + bs[l]
        x = x0 * proj + x
    return x
```

```python
import jax
import jax.numpy as jnp
from jax import lax
import jax.experimental.pallas as pl
import jax.experimental.pallas.tpu as pltpu

_TM = 512


def _kernel(x0_ref, w0_ref, w_hbm, b_ref, o_ref, w_vm, sems):
    L = w_hbm.shape[0]
    i = pl.program_id(0)

    def wcopy(l):
        return pltpu.make_async_copy(w_hbm.at[l], w_vm.at[l - 1], sems.at[l - 1])

    @pl.when(i == 0)
    def _():
        for l in range(1, L):
            wcopy(l).start()
        x0b = x0_ref[...]
        x0 = x0b.astype(jnp.float32)
        p = jnp.dot(x0b, w0_ref[0], preferred_element_type=jnp.float32)
        p = p + b_ref[pl.ds(0, 1), :].astype(jnp.float32)
        o_ref[...] = (x0 * p + x0).astype(o_ref.dtype)

        def body(l, c):
            wcopy(l).wait()
            xb = o_ref[...]
            sel = lax.broadcasted_iota(jnp.int32, b_ref.shape, 0) == l
            brow = jnp.sum(jnp.where(sel, b_ref[...].astype(jnp.float32), 0.0), axis=0, keepdims=True)
            p = jnp.dot(xb, w_vm[l - 1], preferred_element_type=jnp.float32) + brow
            o_ref[...] = (x0_ref[...].astype(jnp.float32) * p + xb.astype(jnp.float32)).astype(o_ref.dtype)
            return c

        lax.fori_loop(1, L, body, 0)

    @pl.when(i > 0)
    def _():
        xb = x0_ref[...]
        x0 = xb.astype(jnp.float32)
        x = x0
        for l in range(L):
            w = w0_ref[0] if l == 0 else w_vm[l - 1]
            p = jnp.dot(xb, w, preferred_element_type=jnp.float32)
            p = p + b_ref[pl.ds(l, 1), :].astype(jnp.float32)
            xb = (x0 * p + x).astype(o_ref.dtype)
            x = xb.astype(jnp.float32)
        o_ref[...] = xb


@jax.jit
def pallas_standalone__cross_network_dcn__recsys_kernel(
    x0: jax.Array,
    ws: jax.Array,
    bs: jax.Array,
):
    B, D = x0.shape
    L = ws.shape[0]
    return pl.pallas_call(
        _kernel,
        grid=(B // _TM,),
        in_specs=[
            pl.BlockSpec((_TM, D), lambda i: (i, 0)),
            pl.BlockSpec((1, D, D), lambda i: (0, 0, 0), pipeline_mode=pl.Buffered(1)),
            pl.BlockSpec(memory_space=pl.ANY),
            pl.BlockSpec((L, D), lambda i: (0, 0), pipeline_mode=pl.Buffered(1)),
        ],
        out_specs=pl.BlockSpec((_TM, D), lambda i: (i, 0)),
        out_shape=jax.ShapeDtypeStruct((B, D), x0.dtype),
        scratch_shapes=[
            pltpu.VMEM((L - 1, D, D), ws.dtype),
            pltpu.SemaphoreType.DMA((L - 1,)),
        ],
        compiler_params=pltpu.CompilerParams(
            dimension_semantics=("arbitrary",),
            vmem_limit_bytes=64 * 2**20,
        ),
    )(x0, ws, ws, bs)
```

```python
import jax
import jax.numpy as jnp
from jax import lax
import jax.experimental.pallas as pl
import jax.experimental.pallas.tpu as pltpu

_TM = 512
_KC = 4
_OC = 2


def _kernel(x_hbm, w_hbm, b_hbm, o_hbm,
            w_vm, x_vm, o_vm, acc, b_raw, b_vm,
            wsem, ksem, xsem, osem, bsem):
    f32 = jnp.float32
    L, D, _ = w_hbm.shape
    tm = x_vm.shape[1]
    nt = x_hbm.shape[0] // tm
    kw = D // _KC
    ow = D // _OC
    dt = o_vm.dtype

    def rows(t):
        return pl.ds(pl.multiple_of(t * tm, tm), tm)

    def k_copies(k):
        ks = pl.ds(k * kw, kw)
        return (
            pltpu.make_async_copy(x_hbm.at[pl.ds(0, tm), ks], x_vm.at[0, :, ks], ksem.at[2 * k]),
            pltpu.make_async_copy(w_hbm.at[0, ks, :], w_vm.at[0, ks, :], ksem.at[2 * k + 1]),
        )

    def w_copy(l):
        return pltpu.make_async_copy(w_hbm.at[l], w_vm.at[l], wsem.at[l])

    def x_copy(t, slot):
        return pltpu.make_async_copy(x_hbm.at[rows(t)], x_vm.at[slot], xsem.at[slot])

    def o_copy(t, slot, c):
        cs = pl.ds(c * ow, ow)
        return pltpu.make_async_copy(
            o_vm.at[slot, :, cs], o_hbm.at[rows(t), cs], osem.at[slot * _OC + c])

    b_copy = pltpu.make_async_copy(b_hbm, b_raw, bsem.at[0])
    b_copy.start()
    for cp in k_copies(0):
        cp.start()
    b_copy.wait()
    b_vm[...] = b_raw[...].astype(f32)

    for k in range(_KC):
        xc, wc = k_copies(k)
        xc.wait()
        if k + 1 < _KC:
            for cp in k_copies(k + 1):
                cp.start()
        if k == 0:
            w_copy(1).start(priority=1)
        wc.wait()
        ks = pl.ds(k * kw, kw)
        p = jnp.dot(x_vm[0, :, ks], w_vm[0, ks, :], preferred_element_type=f32)
        p = p + (b_vm[pl.ds(0, 1), :] if k == 0 else acc[...])
        if k < _KC - 1:
            acc[...] = p
        else:
            x0 = x_vm[0].astype(f32)
            o_vm[(L + 1) % 2] = (x0 * p + x0).astype(dt)

    def first_tile_layer(l, carry):
        w_copy(l).wait()

        @pl.when(l + 1 < L)
        def _():
            w_copy(l + 1).start()

        @pl.when(l + 1 == L)
        def _():
            x_copy(1, 1).start()

        cur = (l + L) % 2
        xb = o_vm[cur]
        p = jnp.dot(xb, w_vm[l], preferred_element_type=f32) + b_vm[pl.ds(l, 1), :]
        o_vm[1 - cur] = (x_vm[0].astype(f32) * p + xb.astype(f32)).astype(dt)
        return carry

    lax.fori_loop(1, L, first_tile_layer, 0)
    for c in range(_OC - 1):
        o_copy(0, 0, c).start()
    x_copy(1, 1).wait()

    def tile(t, carry):
        slot = t % 2
        nxt = jnp.minimum(t + 1, nt - 1)
        xb = x_vm[slot]
        x0 = xb.astype(f32)
        x = x0
        x_copy(nxt, 1 - slot).start()
        o_copy(t - 1, 1 - slot, _OC - 1).start()
        for l in range(L - 1):
            p = jnp.dot(xb, w_vm[l], preferred_element_type=f32) + b_vm[pl.ds(l, 1), :]
            xb = (x0 * p + x).astype(dt)
            x = xb.astype(f32)
        for c in range(_OC):
            cs = slice(c * ow, (c + 1) * ow)
            p = jnp.dot(xb, w_vm[L - 1, :, cs], preferred_element_type=f32)
            p = p + b_vm[pl.ds(L - 1, 1), cs]
            o_vm[slot, :, cs] = (x0[:, cs] * p + x[:, cs]).astype(dt)
            if c < _OC - 1:
                o_copy(t, slot, c).start()
        x_copy(nxt, 1 - slot).wait()
        for c in range(_OC):
            o_copy(t - 1, 1 - slot, c).wait()
        return carry

    lax.fori_loop(1, nt, tile, 0)
    o_copy(nt - 1, (nt - 1) % 2, _OC - 1).start()
    for c in range(_OC):
        o_copy(nt - 1, (nt - 1) % 2, c).wait()


def _cross_network(x0, ws, bs, tm=_TM, interpret=False):
    B, D = x0.shape
    L = ws.shape[0]
    assert B % tm == 0 and B // tm >= 2 and L >= 2
    assert D % (128 * _KC) == 0 and D % (128 * _OC) == 0
    hbm = pl.BlockSpec(memory_space=pl.ANY)
    return pl.pallas_call(
        _kernel,
        in_specs=[hbm, hbm, hbm],
        out_specs=hbm,
        out_shape=jax.ShapeDtypeStruct((B, D), x0.dtype),
        scratch_shapes=[
            pltpu.VMEM((L, D, D), ws.dtype),
            pltpu.VMEM((2, tm, D), x0.dtype),
            pltpu.VMEM((2, tm, D), x0.dtype),
            pltpu.VMEM((tm, D), jnp.float32),
            pltpu.VMEM((L, D), bs.dtype),
            pltpu.VMEM((L, D), jnp.float32),
            pltpu.SemaphoreType.DMA((L,)),
            pltpu.SemaphoreType.DMA((2 * _KC,)),
            pltpu.SemaphoreType.DMA((2,)),
            pltpu.SemaphoreType.DMA((2 * _OC,)),
            pltpu.SemaphoreType.DMA((1,)),
        ],
        compiler_params=pltpu.CompilerParams(vmem_limit_bytes=64 * 2**20),
        interpret=interpret,
    )(x0, ws, bs)


@jax.jit
def pallas_standalone__cross_network_dcn__recsys_kernel(
    x0: jax.Array,
    ws: jax.Array,
    bs: jax.Array,
):
    return _cross_network(x0, ws, bs)
```
